```python
import os as _os
_os.environ.setdefault("JAX_PLATFORMS", "cpu")
import jax
import jax.numpy as jnp

def _softmax(x, axis=-1):
    return jax.nn.softmax(x, axis=axis)
def _gelu(x):
    return jax.nn.gelu(x, approximate=True)
def _silu(x):
    return jax.nn.silu(x)
def _sigmoid(x):
    return jax.nn.sigmoid(x)
def _layernorm(x, axis=-1, eps=1e-5):
    m = jnp.mean(x, axis=axis, keepdims=True)
    v = jnp.var(x, axis=axis, keepdims=True)
    return (x - m) / jnp.sqrt(v + eps)
def _scatter_add(tgt, idx, src, axis=0):
    return tgt.at[idx].add(src)
def _segment_sum(src, seg, n):
    return jax.ops.segment_sum(src, seg, n)
class _Rng:
    def __init__(self, key):
        self._k = key
    def _next(self):
        self._k, sub = jax.random.split(self._k)
        return sub
    def normal(self, shape):
        return jax.random.normal(self._next(), shape, dtype=jnp.bfloat16)
    def randint(self, lo, hi, shape):
        return jax.random.randint(self._next(), shape, lo, hi, dtype=jnp.int32)
    def uniform(self, shape, lo=0.0, hi=1.0):
        return jax.random.uniform(self._next(), shape, jnp.bfloat16, lo, hi)
    def permutation(self, n):
        return jax.random.permutation(self._next(), n)


kernel_name = 'sequential_preLN__linear_kernel_hedgehog__geglu_ffn__prompt'

def setup_inputs():
    _rng = _Rng(jax.random.key(int.from_bytes(__import__("os").urandom(4), "little")))
    _w = (lambda a: (lambda t: t.astype(jnp.bfloat16) if jnp.issubdtype(t.dtype, jnp.floating) else t)(jnp.asarray(a)))
    def _A_setup():
        B, S, D, H = 1, 2048, 640, 32
        Dh = D // H
        return {
            "x": _w((lambda *s: _rng.normal(s) * 0.05)(B, S, D)),
            "wqkv": _w((lambda *s: _rng.normal(s) * 0.2)(D, 3 * D)),
            "w_phi": _w((lambda *s: _rng.normal(s) * 0.2)(H, Dh, Dh) * (Dh ** -0.5)),
            "wo": _w((lambda *s: _rng.normal(s) * 0.05)(D, D)),
        }
    _A_in = _A_setup()

    def _B_setup():
        B, S, D, F = 1, 2048, 640, 1536
        return {
            "x": _w((lambda *s: _rng.normal(s) * 0.05)(B, S, D)),
            "w_gate": _w((lambda *s: _rng.normal(s) * 0.05)(D, F)),
            "w_up": _w((lambda *s: _rng.normal(s) * 0.05)(D, F)),
            "w_down": _w((lambda *s: _rng.normal(s) * 0.05)(F, D)),
        }
    _B_in = _B_setup()

    return {
        "A_x": _A_in["x"],
        "A_wqkv": _A_in["wqkv"],
        "A_w_phi": _A_in["w_phi"],
        "A_wo": _A_in["wo"],
        "B_x": _B_in["x"],
        "B_w_gate": _B_in["w_gate"],
        "B_w_up": _B_in["w_up"],
        "B_w_down": _B_in["w_down"],
    }

def reference(A_x, A_wqkv, A_w_phi, A_wo, B_x, B_w_gate, B_w_up, B_w_down):
    def _A_ref(x, wqkv, w_phi, wo):
        B, S, D = x.shape
        H = 32; Dh = D // H
        qkv = (lambda x, *d: x.transpose(*d))((x @ wqkv).reshape(B, S, 3, H, Dh), 2, 0, 3, 1, 4)
        q, k, v = qkv[0], qkv[1], qkv[2]
        pq = jnp.einsum("bhsd,hdf->bhsf", q, w_phi)
        pk = jnp.einsum("bhsd,hdf->bhsf", k, w_phi)
        phi_q = jnp.concatenate([_softmax(pq, axis=-1), _softmax(-pq, axis=-1)], axis=-1)
        phi_k = jnp.concatenate([_softmax(pk, axis=-1), _softmax(-pk, axis=-1)], axis=-1)
        kv = jnp.einsum("bhsf,bhsd->bhfd", phi_k, v)
        z  = jnp.einsum("bhsf->bhf", phi_k)
        num = jnp.einsum("bhqf,bhfd->bhqd", phi_q, kv)
        den = jnp.einsum("bhqf,bhf->bhq", phi_q, z)[..., None] + 1e-6
        o = num / den
        return (lambda x, *d: x.transpose(*d))(o, 0, 2, 1, 3).reshape(B, S, D) @ wo

    def _B_ref(x, w_gate, w_up, w_down):
        return (_gelu(x @ w_gate) * (x @ w_up)) @ w_down

    x = A_x
    h = x + _A_ref(_layernorm(x, axis=-1), A_wqkv, A_w_phi, A_wo)
    h2 = h + _B_ref(_layernorm(h, axis=-1), B_w_gate, B_w_up, B_w_down)
    return h2
```

```python
import math

import jax
import jax.numpy as jnp
from jax import lax
import jax.experimental.pallas as pl
import jax.experimental.pallas.tpu as pltpu

_F32 = jnp.float32
_BF16 = jnp.bfloat16

_HG = 2
_T = 256
_FC = 512
_MH = 256
_PR = 16

_NN = (((1,), (0,)), ((), ()))
_NT = (((1,), (1,)), ((), ()))
_TN = (((0,), (0,)), ((), ()))
_LOG2E = math.log2(math.e)


def _dot(a, b, dims=_NN):
    return lax.dot_general(a, b, dims, preferred_element_type=_F32)


def _iota(shape, axis):
    return lax.broadcasted_iota(jnp.int32, shape, axis)


def _layernorm(x):
    m = jnp.mean(x, axis=-1, keepdims=True)
    c = x - m
    v = jnp.mean(c * c, axis=-1, keepdims=True)
    return c * lax.rsqrt(v + 1e-5)


def _gelu2(x):
    c = math.sqrt(2.0 / math.pi)
    return x * (1.0 + jnp.tanh(x * (c + (c * 0.044715) * (x * x))))


def _split_lhs(a11, a12, a21, a22):
    return (a11 + a22, a21 + a22, a11, a22, a11 + a12, a21 - a11, a12 - a22)


def _split_rhs(b11, b12, b21, b22):
    return (b11 + b22, b11, b12 - b22, b21 - b11, b22, b11 + b12, b21 + b22)


_RHS_SUMS = (0, 2, 3, 5, 6)


def _join(m1, m2, m3, m4, m5, m6, m7):
    return m1 + m4 - m5 + m7, m3 + m5, m2 + m4, m1 - m2 + m3 + m6


def _blocks(c11, c12, c21, c22):
    return jnp.concatenate([jnp.concatenate([c11, c12], axis=1),
                            jnp.concatenate([c21, c22], axis=1)], axis=0)


def _per_head(x, reduce, combine):
    r = reduce(x, axis=0)
    shift = 4
    while shift >= _HG:
        r = combine(r, pltpu.roll(r, shift, 0))
        shift //= 2
    return r[None]


def _head_sum(x):
    return _per_head(x, jnp.sum, jnp.add)


def _dual_exp(p):
    ep = jnp.exp2(p - _per_head(p, jnp.max, jnp.maximum))
    en = jnp.exp2(_per_head(p, jnp.min, jnp.minimum) - p)
    return ep, en


def _recip(s):
    r = pl.reciprocal(s, approx=True)
    return r * (2.0 - s * r)


def _span(start, size, align):
    if not isinstance(start, int):
        start = pl.multiple_of(start, align)
    return pl.ds(start, size)


def _tile(i, t):
    return _span(i * t, t, t)


def _kernel(
    x_hbm, wqkv_hbm, wphi_hbm, wo_hbm, wg_hbm, wu_hbm, wd_hbm,
    out_hbm,
    x_v, wqkv_v, wphi_v, wo_v, wg_v, wu_v, wd_v,
    wcat_v, wq_v, wkv_v,
    xn_v, kv_acc, z_v, kvt_v, h_v, hn_v, hs_v, out_v,
    sem_x, sem_w, sem_f, sem_o,
):
    S, D = x_hbm.shape
    Dh, _, H = wphi_hbm.shape
    F = wg_hbm.shape[1]
    T, FC, MH = _T, _FC, _MH
    TH, FH, DH = T // 2, FC // 2, D // 2
    G = H // _HG
    R = _HG * Dh
    NV = R // 8
    NC = F // FC
    n = S // T

    def x_copy(i, lo, hi):
        rows = pl.ds(lo * T, (hi - lo) * T)
        return pltpu.make_async_copy(x_hbm.at[rows], x_v.at[rows], sem_x.at[i])

    def qkv_copy(i, lo, hi):
        cols = pl.ds(lo, hi - lo)
        return pltpu.make_async_copy(
            wqkv_hbm.at[:, cols], wqkv_v.at[:, cols], sem_w.at[i])

    def ffn_copies(c):
        f = _tile(c, FC)
        return [pltpu.make_async_copy(src, dst, sem_f.at[3 * c + m])
                for m, (src, dst) in enumerate((
                    (wg_hbm.at[:, f], wg_v.at[pl.ds(0, D), f]),
                    (wu_hbm.at[:, f], wu_v.at[pl.ds(0, D), f]),
                    (wd_hbm.at[f], wd_v.at[f])))]

    def out_copy(i, rows):
        return pltpu.make_async_copy(out_v.at[rows], out_hbm.at[rows], sem_o.at[i])

    phi_copy = pltpu.make_async_copy(wphi_hbm, wphi_v, sem_w.at[0])
    wo_copy = pltpu.make_async_copy(wo_hbm, wo_v, sem_w.at[1])
    q_copy, v_copy = qkv_copy(2, 0, D), qkv_copy(3, 2 * D, 3 * D)
    ka_copy, kb_copy = qkv_copy(4, D, D + 384), qkv_copy(5, D + 384, 2 * D)
    x0_copy, x1_copy, x2_copy = [x_copy(i, i, i + 1) for i in range(3)]
    x3_copy = x_copy(3, 3, n)

    for c in (phi_copy, x0_copy, ka_copy, kb_copy, x1_copy):
        c.start()

    r = _iota((D, D), 0)
    place = jnp.where(_iota((D, D), 1) == (r % H) * Dh + r // H, 1.0, 0.0)
    place = place.astype(_BF16)
    expand = jnp.where(_iota((R, 32), 0) // _HG == _iota((R, 32), 1), 1.0, 0.0)
    wcat_v[...] = jnp.zeros(wcat_v.shape, _F32)
    phi_copy.wait()
    for d in range(Dh):
        wcat_v[:Dh, d * H:(d + 1) * H] = wphi_v[d].astype(_F32)
    ft = _dot(wcat_v[...].astype(_BF16), place)
    ft = _dot(expand.astype(_BF16), ft.astype(_BF16))
    head_lo = (_iota((R, 128), 0) % _HG) * Dh
    lane = _iota((R, 128), 1)

    def fold_part(j, t, parts):
        gs = [g for g in range(G) if g * R < (t + 1) * 128 and (g + 1) * R > t * 128]
        pt = []
        for g in gs:
            lo = head_lo + (g * R - t * 128)
            own = (lane >= lo) & (lane < lo + Dh)
            pt.append(jnp.where(own, ft[:, t * 128:(t + 1) * 128], 0.0))
        pt = jnp.concatenate(pt, axis=0).astype(_BF16)
        res = _dot(pt, wqkv_v[:, j * D + t * 128:j * D + (t + 1) * 128], _NT)
        for m, g in enumerate(gs):
            parts[g].append(res[m * R:(m + 1) * R])

    def folded(parts):
        return _LOG2E * jnp.concatenate([sum(p[1:], p[0]) for p in parts], axis=0)

    def put_kv(j, wt):
        for c in range(2):
            wkv_v[c, j * DH:(j + 1) * DH] = wt[c * DH:(c + 1) * DH].astype(_F32)

    def up_block(m, c):
        if m in _RHS_SUMS:
            k = _RHS_SUMS.index(m)
            return D + MH * (k // 2), (k % 2) * (F // 2) + c * FH
        return (0, c * FC) if m == 1 else (MH, c * FC + FH)

    def down_block(m, c):
        if m in _RHS_SUMS:
            k = _RHS_SUMS.index(m)
            return F + (F // 2) * (k // 2) + c * FH, (k % 2) * MH
        return (c * FC, 0) if m == 1 else (c * FC + FH, MH)

    def block_sums(w_v, dst, src, rows, cols):
        def at(r, c):
            return _span(r, _PR, _PR), _span(c, cols, 128)

        for r0 in range(0, rows, _PR):
            ops = _split_rhs(*[w_v[at(r + r0, c)].astype(_F32) for r, c in src])
            for m in _RHS_SUMS:
                r, c = dst(m)
                w_v[at(r + r0, c)] = ops[m].astype(_BF16)

    def prepare_ffn(c):
        for w_v in (wg_v, wu_v):
            block_sums(w_v, lambda m: up_block(m, c),
                       [(r, c * FC + k) for r in (0, MH) for k in (0, FH)], MH, FH)
        block_sums(wd_v, lambda m: down_block(m, c),
                   [(c * FC + r, k) for r in (0, FH) for k in (0, MH)], FH, MH)

    def norm_x(i):
        xn_v[_tile(i, T)] = _layernorm(x_v[_tile(i, T)].astype(_F32)).astype(_BF16)

    def kv_update(c, pk, vt, first=False):
        for m in range(G // 2):
            g, rows = c * (G // 2) + m, slice(m * R, (m + 1) * R)
            ep, en = _dual_exp(pk[rows].reshape(NV, 8, T))
            pp = ep * _recip(_head_sum(ep))
            pn = en * _recip(_head_sum(en))
            phi = jnp.concatenate([pp, pn], axis=0).reshape(2 * R, T)
            v = jnp.concatenate([vt[rows], jnp.ones((8, T), _F32)], axis=0)
            kv = _dot(v, phi, _NT)
            kv_acc[g] = kv if first else kv_acc[g] + kv

    def kv_step(i):
        xn = xn_v[_tile(i, T)]
        proj = [_dot(wkv_v[c], xn, _NT) for c in range(2)]
        for c, p in enumerate(proj):
            kv_update(c, p[:DH], p[DH:])

    def project(j, i):
        w = jnp.concatenate([wkv_v[c, j * DH:(j + 1) * DH] for c in range(2)], axis=0)
        return _dot(w, xn_v[_tile(i, T)], _NT)

    def q_proj(i):
        return _dot(wq_v[...], xn_v[_tile(i, T)], _NT)

    parts = [[] for _ in range(G)]
    x0_copy.wait()
    v_copy.start()
    x2_copy.start()
    norm_x(0)
    ka_copy.wait()
    x3_copy.start()
    for t in range(3):
        fold_part(1, t, parts)
    kb_copy.wait()
    for t in range(3, D // 128):
        fold_part(1, t, parts)
    put_kv(0, folded(parts))
    x1_copy.wait()
    pk0 = project(0, 0)
    norm_x(1)
    v_copy.wait()
    x2_copy.wait()
    for k in range(NC):
        for c in ffn_copies(k):
            c.start()
    pk1 = project(0, 1)
    put_kv(1, wqkv_v[:, 2 * D:].T)
    norm_x(2)
    for i, pk in enumerate((pk0, pk1)):
        vt = project(1, i)
        for c in range(2):
            kv_update(c, pk[c * DH:(c + 1) * DH], vt[c * DH:(c + 1) * DH], i == 0)
    x3_copy.wait()
    for i in range(2, n - 1 - NC):
        kv_step(i)
        norm_x(i + 1)
    q_copy.start()
    wo_copy.start()

    def pass1(k, carry):
        for c in ffn_copies(k):
            c.wait()
        kv_step(n - 1 - NC + k)
        norm_x(n - NC + k)
        prepare_ffn(k)
        return carry

    lax.fori_loop(0, NC, pass1, 0)
    q_copy.wait()
    wo_copy.wait()
    parts = [[] for _ in range(G)]
    for t in range(D // 128):
        fold_part(0, t, parts)
    wq_v[...] = folded(parts)
    kv_step(n - 1)
    pq0 = q_proj(0)

    lo = (_iota((R, 2 * R), 1) % _HG) * Dh
    row = _iota((R, 2 * R), 0)
    same = (row >= lo) & (row < lo + Dh)
    for g in range(G):
        kvt_v[g] = jnp.where(same, kv_acc[g, :R], 0.0)
        z_v[g] = jnp.broadcast_to(kv_acc[g, R:R + 1], (128, 2 * R)).T

    def attend(pq):
        ots = []
        for g in range(G):
            ep, en = _dual_exp(pq[g * R:(g + 1) * R].reshape(NV, 8, T))
            z = jnp.concatenate([z_v[g]] * (T // 128), axis=-1)
            z = z.reshape(2 * NV, 8, T)
            ip = _recip(_head_sum(ep))
            im = _recip(_head_sum(en))
            den = _head_sum(ep * z[:NV]) * ip + _head_sum(en * z[NV:]) * im
            inv = 1.0 / (den + 1e-6)
            phi = jnp.concatenate([ep * (ip * inv), en * (im * inv)], axis=0)
            ots.append(_dot(kvt_v[g], phi.reshape(2 * R, T)))
        return jnp.concatenate(ots, axis=0).astype(_BF16)

    def out_proj(i, ot):
        h = x_v[_tile(i, T)].astype(_F32) + _dot(ot, wo_v[...], _TN)
        h_v[_tile(i, T)] = h
        hn = _layernorm(h)
        hn_v[_tile(i, T)] = hn[:, 2 * MH:].astype(_BF16)
        ops = _split_lhs(hn[:TH, :MH], hn[:TH, MH:2 * MH],
                         hn[TH:, :MH], hn[TH:, MH:2 * MH])
        for m, a in enumerate(ops):
            hs_v[m, _tile(i, TH)] = a.astype(_BF16)

    def up_proj(i, c, w_v):
        y = _dot(hn_v[_tile(i, T)], w_v[2 * MH:D, c * FC:(c + 1) * FC])
        ms = []
        for m in range(7):
            r, k = up_block(m, c)
            ms.append(_dot(hs_v[m, _tile(i, TH)], w_v[r:r + MH, k:k + FH]))
        ys = (y[:TH, :FH], y[:TH, FH:], y[TH:, :FH], y[TH:, FH:])
        return [a + b for a, b in zip(ys, _join(*ms))]

    def glu(i, c):
        act = [_gelu2(g) * u
               for g, u in zip(up_proj(i, c, wg_v), up_proj(i, c, wu_v))]
        return (_blocks(*act).astype(_BF16),
                [a.astype(_BF16) for a in _split_lhs(*act)])

    def down_rest(acts):
        whole = jnp.concatenate([a for a, _ in acts], axis=1)
        return _dot(whole, wd_v[:F, 2 * MH:])

    def down_product(acts, m):
        w = [wd_v[r:r + FH, k:k + MH]
             for r, k in (down_block(m, c) for c in range(NC))]
        return _dot(jnp.concatenate([ops[m] for _, ops in acts], axis=1),
                    jnp.concatenate(w, axis=0))

    def emit(i, rows, y):
        out_v[rows] = (h_v[rows] + 0.5 * y).astype(out_v.dtype)
        out_copy(i, rows).start()

    out_proj(0, attend(pq0))

    def pass2(i, carry):
        acts = [glu(i, 0)]
        pq = q_proj(i + 1)
        acts.append(glu(i, 1))
        ot = attend(pq)
        acts += [glu(i, c) for c in range(2, NC)]
        out_proj(i + 1, ot)
        ms = [down_product(acts, m) for m in range(7)]
        emit(i, _tile(i, T),
             jnp.concatenate([_blocks(*_join(*ms)), down_rest(acts)], axis=1))
        return carry

    lax.fori_loop(0, n - 1, pass2, 0)

    acts = [glu(n - 1, c) for c in range(NC)]
    rest = down_rest(acts)
    upper, lower = pl.ds((n - 1) * T, TH), pl.ds((n - 1) * T + TH, TH)
    m1, m2, m3, m4, m6 = [down_product(acts, m) for m in (0, 1, 2, 3, 5)]
    emit(n, lower, jnp.concatenate([m2 + m4, m1 - m2 + m3 + m6, rest[TH:]], axis=1))
    m5, m7 = down_product(acts, 4), down_product(acts, 6)
    emit(n - 1, upper,
         jnp.concatenate([m1 + m4 - m5 + m7, m3 + m5, rest[:TH]], axis=1))
    for i in range(n - 1):
        out_copy(i, _tile(i, T)).wait()
    out_copy(n, lower).wait()
    out_copy(n - 1, upper).wait()


@jax.jit
def pallas_sequential_preLN__linear_kernel_hedgehog__geglu_ffn__prompt_kernel(
    A_x: jax.Array,
    A_wqkv: jax.Array,
    A_w_phi: jax.Array,
    A_wo: jax.Array,
    B_x: jax.Array,
    B_w_gate: jax.Array,
    B_w_up: jax.Array,
    B_w_down: jax.Array,
):
    del B_x
    B, S, D = A_x.shape
    H, Dh, _ = A_w_phi.shape
    F = B_w_gate.shape[1]
    assert (B, S, D, H, Dh, F) == (1, 2048, 640, 32, 20, 1536)
    G, R = H // _HG, _HG * Dh

    out = pl.pallas_call(
        _kernel,
        in_specs=[pl.BlockSpec(memory_space=pl.ANY)] * 7,
        out_specs=pl.BlockSpec(memory_space=pl.ANY),
        out_shape=jax.ShapeDtypeStruct((S, D), A_x.dtype),
        scratch_shapes=[
            pltpu.VMEM((S, D), A_x.dtype),
            pltpu.VMEM((D, 3 * D), A_wqkv.dtype),
            pltpu.VMEM((Dh, Dh, H), A_w_phi.dtype),
            pltpu.VMEM((D, D), A_wo.dtype),
            pltpu.VMEM((D + 3 * _MH, F), B_w_gate.dtype),
            pltpu.VMEM((D + 3 * _MH, F), B_w_up.dtype),
            pltpu.VMEM((F + 3 * F // 2, D), B_w_down.dtype),
            pltpu.VMEM((32, D), _F32),
            pltpu.VMEM((D, D), _F32),
            pltpu.VMEM((2, D, D), _F32),
            pltpu.VMEM((S, D), _BF16),
            pltpu.VMEM((G, R + 8, 2 * R), _F32),
            pltpu.VMEM((G, 2 * R, 128), _F32),
            pltpu.VMEM((G, R, 2 * R), _F32),
            pltpu.VMEM((S, D), _F32),
            pltpu.VMEM((S, D - 2 * _MH), _BF16),
            pltpu.VMEM((7, S // 2, _MH), _BF16),
            pltpu.VMEM((S, D), A_x.dtype),
            pltpu.SemaphoreType.DMA((4,)),
            pltpu.SemaphoreType.DMA((6,)),
            pltpu.SemaphoreType.DMA((3 * (F // _FC),)),
            pltpu.SemaphoreType.DMA((S // _T + 1,)),
        ],
        compiler_params=pltpu.CompilerParams(vmem_limit_bytes=100 * 1024 * 1024),
    )(A_x.reshape(S, D), A_wqkv, A_w_phi.transpose(1, 2, 0), A_wo,
      B_w_gate, B_w_up, B_w_down)
    return out.reshape(B, S, D)
```
